```python
import os as _os
_os.environ.setdefault("JAX_PLATFORMS", "cpu")
import jax
import jax.numpy as jnp

def _softmax(x, axis=-1):
    return jax.nn.softmax(x, axis=axis)
def _gelu(x):
    return jax.nn.gelu(x, approximate=True)
def _silu(x):
    return jax.nn.silu(x)
def _sigmoid(x):
    return jax.nn.sigmoid(x)
def _layernorm(x, axis=-1, eps=1e-5):
    m = jnp.mean(x, axis=axis, keepdims=True)
    v = jnp.var(x, axis=axis, keepdims=True)
    return (x - m) / jnp.sqrt(v + eps)
def _scatter_add(tgt, idx, src, axis=0):
    return tgt.at[idx].add(src)
def _segment_sum(src, seg, n):
    return jax.ops.segment_sum(src, seg, n)
class _Rng:
    def __init__(self, key):
        self._k = key
    def _next(self):
        self._k, sub = jax.random.split(self._k)
        return sub
    def normal(self, shape):
        return jax.random.normal(self._next(), shape, dtype=jnp.bfloat16)
    def randint(self, lo, hi, shape):
        return jax.random.randint(self._next(), shape, lo, hi, dtype=jnp.int32)
    def uniform(self, shape, lo=0.0, hi=1.0):
        return jax.random.uniform(self._next(), shape, jnp.bfloat16, lo, hi)
    def permutation(self, n):
        return jax.random.permutation(self._next(), n)


kernel_name = 'standalone__mha_softmax__near_ridge'

def setup_inputs():
    _rng = _Rng(jax.random.key(int.from_bytes(__import__("os").urandom(4), "little")))
    _w = (lambda a: (lambda t: t.astype(jnp.bfloat16) if jnp.issubdtype(t.dtype, jnp.floating) else t)(jnp.asarray(a)))
    B, H, Sq, Sk, D = 8, 32, 384, 512, 128
    return {
        "q": _w((lambda *s: _rng.normal(s) * 0.4)(B, H, Sq, D)),
        "k": _w((lambda *s: _rng.normal(s) * 0.4)(B, H, Sk, D)),
        "v": _w((lambda *s: _rng.normal(s) * 0.05)(B, H, Sk, D)),
    }

def reference(q, k, v):
    scale = q.shape[-1] ** -0.5
    scores = jnp.einsum("bhqd,bhkd->bhqk", q, k) * scale
    p = _softmax(scores, axis=-1)
    return jnp.einsum("bhqk,bhkd->bhqd", p, v)
```

```python
import functools

import jax
import jax.numpy as jnp
from jax import lax
import jax.experimental.pallas as pl
import jax.experimental.pallas.tpu as pltpu

LOG2E = 1.4426950408889634

HEADS_PER_STEP = 8
READ_UNIT = 2
READ_RATE = 10
PRELOAD = 12
RING = 128
WRITE_UNIT = 4
WRITE_RATE = 8
WRITE_DELAY = 193
CHUNK = 128


def _attend(q, k, v, c):
    s = lax.dot_general(q, k, (((1,), (1,)), ((), ())), preferred_element_type=jnp.float32)
    m = jnp.max(s, axis=-1, keepdims=True)
    p = jnp.exp2((s - m) * c)
    l = jnp.sum(p, axis=-1, keepdims=True)
    o = jnp.dot(p.astype(v.dtype), v, preferred_element_type=jnp.float32)
    r = pl.reciprocal(l, approx=True)
    r = r * (2.0 - l * r)
    return o * r


@jax.jit
def pallas_standalone__mha_softmax__near_ridge_kernel(
    q: jax.Array,
    k: jax.Array,
    v: jax.Array,
):
    B, H, Sq, D = q.shape
    Sk = k.shape[2]
    NH = B * H
    hb, U, R, wU, C = HEADS_PER_STEP, READ_UNIT, RING, WRITE_UNIT, CHUNK
    n = NH // hb
    scale = (D ** -0.5) * LOG2E
    seqs = (Sq, Sk, Sk)
    runit = [(t, c, u) for c in range(max(seqs) // C) for t in range(3) if c < seqs[t] // C for u in range(U)]
    wunit = [(c, u) for c in range(Sq // C) for u in range(wU)]
    ndr = len(runit) * (READ_RATE // U)
    ndw = len(wunit) * WRITE_RATE
    nwu = NH // wU
    tail0 = min(nwu, max(0, n * WRITE_RATE - WRITE_DELAY))

    def kernel_function(q_hbm, k_hbm, v_hbm, o_hbm, qb, kb, vb, ob, rsem, wsem):
        hbm = (q_hbm, k_hbm, v_hbm)
        bufs = (qb, kb, vb)

        def rd_start(j0, d):
            t, c, u = runit[d]
            j = j0 + u
            pltpu.make_async_copy(
                hbm[t].at[j % B, j // B, pl.ds(c * C, C)],
                bufs[t].at[j % R, pl.ds(c * C, C)],
                rsem.at[(j0 % R) // U],
            ).start(priority=d % 2)

        def rd_wait(j0):
            sl = pl.multiple_of(j0 % R, U)
            for t in range(3):
                dst = bufs[t].at[pl.ds(sl, U)]
                pltpu.make_async_copy(dst, dst, rsem.at[(j0 % R) // U]).wait()

        def wr_start(j0, d):
            c, u = wunit[d]
            j = j0 + u
            pltpu.make_async_copy(
                ob.at[j, pl.ds(c * C, C)],
                o_hbm.at[j % B, j // B, pl.ds(c * C, C)],
                wsem,
            ).start(priority=d % 2)

        for j0 in range(0, PRELOAD, U):
            for d in range(len(runit)):
                rd_start(j0, d)

        def body(it, _):
            for u in range(0, hb, U):
                rd_wait(it * hb + u)
            pending = None
            for s in range(hb):
                i = it * hb + s
                for d in range(ndr * s // hb, ndr * (s + 1) // hb):
                    j0 = PRELOAD + it * READ_RATE + (d // len(runit)) * U
                    pl.when(j0 < NH)(
                        functools.partial(rd_start, jnp.minimum(j0, NH - U), d % len(runit)))
                for d in range(ndw * s // hb, ndw * (s + 1) // hb):
                    w = it * WRITE_RATE - WRITE_DELAY + d // len(wunit)
                    pl.when(jnp.logical_and(w >= 0, w < nwu))(
                        functools.partial(wr_start, jnp.clip(w, 0, nwu - 1) * wU, d % len(wunit)))
                if pending is not None:
                    ob[i - 1] = pending
                ld = lambda ref: pltpu.bitcast(ref.bitcast(jnp.uint32)[i % R], jnp.bfloat16)
                pending = _attend(ld(qb), ld(kb), ld(vb), scale).astype(ob.dtype)
            ob[it * hb + hb - 1] = pending

        lax.fori_loop(0, n, body, None)
        for w in range(tail0, nwu):
            for d in range(len(wunit)):
                wr_start(w * wU, d)
        pltpu.make_async_copy(ob, ob, wsem).wait()

    return pl.pallas_call(
        kernel_function,
        in_specs=[pl.BlockSpec(memory_space=pl.ANY)] * 3,
        out_specs=pl.BlockSpec(memory_space=pl.ANY),
        out_shape=jax.ShapeDtypeStruct(q.shape, q.dtype),
        scratch_shapes=[
            pltpu.VMEM((R, Sq, D), q.dtype),
            pltpu.VMEM((R, Sk, D), k.dtype),
            pltpu.VMEM((R, Sk, D), v.dtype),
            pltpu.VMEM((NH, Sq, D), q.dtype),
            pltpu.SemaphoreType.DMA((R // U,)),
            pltpu.SemaphoreType.DMA(()),
        ],
        compiler_params=pltpu.CompilerParams(
            vmem_limit_bytes=100 * 1024 * 1024,
            disable_bounds_checks=True,
            disable_semaphore_checks=True,
            flags={"XLA_TPU_MAX_INSTS_TO_PREDICATE": 65536},
        ),
    )(q, k, v)
```

```python
import functools

import jax
import jax.numpy as jnp
from jax import lax
import jax.experimental.pallas as pl
import jax.experimental.pallas.tpu as pltpu

LOG2E = 1.4426950408889634

UNIT = 2
UNIT_SLOTS = 5
PRELOAD_UNITS = 8
READ_STEPS = 25
RING = 16
READ_ROWS = 128
WRITE_ROWS = 128
WRITE_HEADS = 4
WRITE_RATE = 5
READ_ORDER = ((1, 0), (2, 0), (0, 0), (1, 1), (1, 2), (2, 1), (0, 1), (2, 2), (1, 3), (2, 3), (0, 2))


def _attend(q, k, v, scale_log2e):
    s = lax.dot_general(q, k, (((1,), (1,)), ((), ())), preferred_element_type=jnp.float32)
    m = jnp.max(s, axis=-1, keepdims=True)
    p = jnp.exp2((s - m) * scale_log2e)
    l = jnp.sum(p, axis=-1, keepdims=True)
    o = jnp.dot(p.astype(v.dtype), v, preferred_element_type=jnp.float32)
    r = pl.reciprocal(l, approx=True)
    r = r * (2.0 - l * r)
    return o * r


@jax.jit
def pallas_standalone__mha_softmax__near_ridge_kernel(
    q: jax.Array,
    k: jax.Array,
    v: jax.Array,
):
    B, H, Sq, D = q.shape
    Sk = k.shape[2]
    assert (B, H, Sq, Sk) == (8, 32, 384, 512) and q.dtype == k.dtype == v.dtype == jnp.bfloat16
    scale_log2e = (D ** -0.5) * LOG2E

    seq = (Sq, Sk, Sk)
    row0 = (0, Sq, Sq + Sk)
    reads = []
    for i in range(0, len(READ_ORDER) - 1, 2):
        for u in range(UNIT):
            reads += [(*READ_ORDER[i], u), (*READ_ORDER[i + 1], u)]
    reads += [(*READ_ORDER[-1], u) for u in range(UNIT)]
    writes = [(b0, r0) for r0 in range(0, Sq, WRITE_ROWS) for b0 in range(0, B, WRITE_HEADS)]
    n_units = B * H // UNIT
    read_slots = len(reads) * UNIT_SLOTS
    unit_rate = pl.cdiv((n_units - PRELOAD_UNITS) * 256, READ_STEPS)

    def batch_of(j):
        return ((j >> 2) & 1) | (j & 2) | ((j & 1) << 2)

    def units_started_before(it):
        return jnp.minimum(n_units, PRELOAD_UNITS + ((unit_rate * it) >> 8))

    def kernel_function(q_hbm, k_hbm, v_hbm, o_hbm, in_buf, out_buf, sems):
        hbm = (q_hbm, k_hbm, v_hbm)
        write_sem = sems.at[RING]

        def start_read(unit, d):
            t, c, u = reads[d]
            j = unit * UNIT + u
            entry = (j >> 3) & (RING - 1)
            pltpu.make_async_copy(
                hbm[t].at[batch_of(j), j >> 3, pl.ds(c * READ_ROWS, READ_ROWS)],
                in_buf.at[entry, j & 7, pl.ds(row0[t] + c * READ_ROWS, READ_ROWS)],
                sems.at[entry],
            ).start(priority=d % 2)

        def start_write(h, d):
            b0, r0 = writes[d]
            where = (pl.ds(b0, WRITE_HEADS), h, pl.ds(r0, WRITE_ROWS))
            pltpu.make_async_copy(out_buf.at[where], o_hbm.at[where], write_sem).start()

        for unit in range(PRELOAD_UNITS):
            for d in range(len(reads)):
                start_read(unit, d)

        def step(it, carry):
            entry = it & (RING - 1)
            pltpu.make_async_copy(in_buf.at[entry], in_buf.at[entry], sems.at[entry]).wait()

            def load(s, t):
                words = in_buf.bitcast(jnp.uint32)[entry, s, pl.ds(row0[t] // 2, seq[t] // 2)]
                return pltpu.bitcast(words, jnp.bfloat16)

            first, end = units_started_before(it), units_started_before(it + 1)
            pending = None
            for s in range(B):
                if s == 1:
                    for i in range(WRITE_RATE):
                        h = (it - READ_STEPS) * WRITE_RATE + i
                        for d in range(len(writes)):
                            pl.when(jnp.logical_and(h >= 0, h < it))(
                                functools.partial(start_write, jnp.clip(h, 0, H - 1), d))
                for d in range(read_slots * s // B, read_slots * (s + 1) // B):
                    unit = first + d // len(reads)
                    pl.when(unit < end)(
                        functools.partial(start_read, jnp.minimum(unit, n_units - 1), d % len(reads)))
                if pending is not None:
                    out_buf[batch_of(s - 1), it] = pending
                o = _attend(load(s, 0), load(s, 1), load(s, 2), scale_log2e)
                pending = o.astype(out_buf.dtype)
            out_buf[batch_of(B - 1), it] = pending
            return carry

        lax.fori_loop(0, H, step, None)

        for h in range(min(H - 1, (H - READ_STEPS) * WRITE_RATE), H):
            for d in range(len(writes)):
                start_write(h, d)
        pltpu.make_async_copy(out_buf, out_buf, write_sem).wait()

    return pl.pallas_call(
        kernel_function,
        in_specs=[pl.BlockSpec(memory_space=pl.ANY)] * 3,
        out_specs=pl.BlockSpec(memory_space=pl.ANY),
        out_shape=jax.ShapeDtypeStruct(q.shape, q.dtype),
        scratch_shapes=[
            pltpu.VMEM((RING, B, Sq + 2 * Sk, D), q.dtype),
            pltpu.VMEM((B, H, Sq, D), q.dtype),
            pltpu.SemaphoreType.DMA((RING + 1,)),
        ],
        compiler_params=pltpu.CompilerParams(
            vmem_limit_bytes=100 * 1024 * 1024,
            disable_bounds_checks=True,
            disable_semaphore_checks=True,
            flags={"XLA_TPU_MAX_INSTS_TO_PREDICATE": 65536},
        ),
    )(q, k, v)
```

```python
import functools

import jax
import jax.numpy as jnp
from jax import lax
import jax.experimental.pallas as pl
import jax.experimental.pallas.tpu as pltpu

LOG2E = 1.4426950408889634

ROWS = 128
RING = 16
FIRST_UNITS = 7
LEAD_UNITS = 8
READ_STEPS = 25
UNITS_PER_STEP = 5
WRITE_BATCHES = 4
WRITE_RATE = 4


def _attend(q, k, v, scale_log2e):
    s = lax.dot_general(q, k, (((1,), (1,)), ((), ())), preferred_element_type=jnp.float32)
    m = jnp.max(s, axis=-1, keepdims=True)
    p = jnp.exp2((s - m) * scale_log2e)
    l = jnp.sum(p, axis=-1, keepdims=True)
    o = jnp.dot(p.astype(v.dtype), v, preferred_element_type=jnp.float32)
    r = pl.reciprocal(l, approx=True)
    r = r * (2.0 - l * r)
    return o * r


@jax.jit
def pallas_standalone__mha_softmax__near_ridge_kernel(
    q: jax.Array,
    k: jax.Array,
    v: jax.Array,
):
    B, H, Sq, D = q.shape
    Sk = k.shape[2]
    assert (B, H, Sq, Sk) == (8, 32, 384, 512), "the copy schedule is laid out for these shapes"
    scale_log2e = (D ** -0.5) * LOG2E

    seq = (Sq, Sk, Sk)
    row0 = (0, Sq, Sq + Sk)
    parts = Sk // ROWS
    q_chunks = B * (Sq // ROWS) // parts
    reads = [(0, i) for i in range(q_chunks)] + [(t, b) for t in (1, 2) for b in range(B)]
    read_slots = len(reads) * UNITS_PER_STEP
    writes = [(b, r) for r in range(0, Sq, ROWS) for b in range(0, B, WRITE_BATCHES)]
    n_units = H * parts
    unit_rate = pl.cdiv((n_units - LEAD_UNITS) * 256, READ_STEPS)

    def units_started_before(h):
        even = jnp.minimum(n_units, LEAD_UNITS + ((unit_rate * h) >> 8))
        return jnp.where(h == 0, FIRST_UNITS, even)

    def kernel_function(q_hbm, k_hbm, v_hbm, o_hbm, in_buf, out_buf, sems):
        hbm = (q_hbm, k_hbm, v_hbm)
        write_sem = sems.at[RING]

        def start_read(unit, d):
            t, i = reads[d]
            h, part = unit >> 2, unit & 3
            if t == 0:
                chunk = q_chunks * part + i
                b, c = chunk & 7, chunk >> 3
            else:
                b, c = i, part
            src, dst = c * ROWS, row0[t] + c * ROWS
            if not isinstance(unit, int):
                src, dst = pl.multiple_of(src, ROWS), pl.multiple_of(dst, ROWS)
            entry = h & (RING - 1)
            pltpu.make_async_copy(
                hbm[t].at[b, h, pl.ds(src, ROWS)],
                in_buf.at[entry, b, pl.ds(dst, ROWS)],
                sems.at[entry],
            ).start(priority=d % 2)

        def start_write(h, d):
            b, r = writes[d]
            where = (pl.ds(b, WRITE_BATCHES), h, pl.ds(r, ROWS))
            pltpu.make_async_copy(out_buf.at[where], o_hbm.at[where], write_sem).start()

        for unit in range(FIRST_UNITS):
            for d in range(len(reads)):
                start_read(unit, d)

        def step(h, carry):
            entry = h & (RING - 1)
            pltpu.make_async_copy(in_buf.at[entry], in_buf.at[entry], sems.at[entry]).wait()

            first, end = units_started_before(h), units_started_before(h + 1)
            pending = None
            for b in range(B):
                if b == 1:
                    for i in range(WRITE_RATE):
                        done = (h - READ_STEPS) * WRITE_RATE + i
                        for d in range(len(writes)):
                            pl.when(jnp.logical_and(done >= 0, done < h))(
                                functools.partial(start_write, jnp.clip(done, 0, H - 1), d))
                for d in range(read_slots * b // B, read_slots * (b + 1) // B):
                    unit = first + d // len(reads)
                    pl.when(unit < end)(functools.partial(
                        start_read, jnp.minimum(unit, n_units - 1), d % len(reads)))
                if pending is not None:
                    out_buf[b - 1, h] = pending
                qkv = [in_buf[entry, b, pl.ds(row0[t], seq[t])] for t in range(3)]
                pending = _attend(*qkv, scale_log2e).astype(out_buf.dtype)
            out_buf[B - 1, h] = pending
            return carry

        lax.fori_loop(0, H, step, None)

        for done in range(min(H - 1, (H - READ_STEPS) * WRITE_RATE), H):
            for d in range(len(writes)):
                start_write(done, d)
        pltpu.make_async_copy(out_buf, o_hbm, write_sem).wait()

    return pl.pallas_call(
        kernel_function,
        in_specs=[pl.BlockSpec(memory_space=pl.ANY)] * 3,
        out_specs=pl.BlockSpec(memory_space=pl.ANY),
        out_shape=jax.ShapeDtypeStruct(q.shape, q.dtype),
        scratch_shapes=[
            pltpu.VMEM((RING, B, Sq + 2 * Sk, D), q.dtype),
            pltpu.VMEM((B, H, Sq, D), q.dtype),
            pltpu.SemaphoreType.DMA((RING + 1,)),
        ],
        compiler_params=pltpu.CompilerParams(
            vmem_limit_bytes=100 * 1024 * 1024,
            disable_bounds_checks=True,
            disable_semaphore_checks=True,
            flags={"XLA_TPU_MAX_INSTS_TO_PREDICATE": 65536},
        ),
    )(q, k, v)
```

```python
import functools

import jax
import jax.numpy as jnp
from jax import lax
import jax.experimental.pallas as pl
import jax.experimental.pallas.tpu as pltpu

LOG2E = 1.4426950408889634

ROWS = 128
RING = 16
FIRST_UNITS = 7
LEAD_UNITS = 8
READ_STEPS = 25
UNITS_PER_STEP = 5
WRITE_ROWS = 96
WRITE_RATE = 5
WRITE_SLOT = 5


def _attend(q, k, v, scale_log2e):
    s = lax.dot_general(q, k, (((1,), (1,)), ((), ())), preferred_element_type=jnp.float32)
    m = jnp.max(s, axis=-1, keepdims=True)
    p = jnp.exp2((s - m) * scale_log2e)
    l = jnp.sum(p, axis=-1, keepdims=True)
    o = jnp.dot(p.astype(v.dtype), v, preferred_element_type=jnp.float32)
    r = pl.reciprocal(l, approx=True)
    r = r * (2.0 - l * r)
    return o * r


@jax.jit
def pallas_standalone__mha_softmax__near_ridge_kernel(
    q: jax.Array,
    k: jax.Array,
    v: jax.Array,
):
    B, H, Sq, D = q.shape
    Sk = k.shape[2]
    assert (B, H, Sq, Sk) == (8, 32, 384, 512), "the copy schedule is laid out for these shapes"
    scale_log2e = (D ** -0.5) * LOG2E

    seq = (Sq, Sk, Sk)
    row0 = (0, Sq, Sq + Sk)
    parts = Sk // ROWS
    q_chunks = B * (Sq // ROWS) // parts
    reads = [(0, i) for i in range(q_chunks)] + [(t, b) for t in (1, 2) for b in range(B)]
    read_slots = len(reads) * UNITS_PER_STEP
    n_units = H * parts
    unit_rate = pl.cdiv((n_units - LEAD_UNITS) * 256, READ_STEPS)

    def units_started_before(h):
        even = jnp.minimum(n_units, LEAD_UNITS + ((unit_rate * h) >> 8))
        return jnp.where(h == 0, FIRST_UNITS, even)

    def kernel_function(q_hbm, k_hbm, v_hbm, o_hbm, in_buf, out_buf, sems):
        hbm = (q_hbm, k_hbm, v_hbm)
        write_sem = sems.at[RING]

        def start_read(unit, d):
            t, i = reads[d]
            h, part = unit >> 2, unit & 3
            if t == 0:
                chunk = q_chunks * part + i
                b, c = chunk & 7, chunk >> 3
            else:
                b, c = i, part
            src, dst = c * ROWS, row0[t] + c * ROWS
            if not isinstance(unit, int):
                src, dst = pl.multiple_of(src, ROWS), pl.multiple_of(dst, ROWS)
            entry = h & (RING - 1)
            pltpu.make_async_copy(
                hbm[t].at[b, h, pl.ds(src, ROWS)],
                in_buf.at[entry, b, pl.ds(dst, ROWS)],
                sems.at[entry],
            ).start(priority=d % 2)

        def start_write(h):
            for r in range(0, Sq, WRITE_ROWS):
                where = (slice(None), h, pl.ds(r, WRITE_ROWS))
                pltpu.make_async_copy(out_buf.at[where], o_hbm.at[where], write_sem).start()

        for unit in range(FIRST_UNITS):
            for d in range(len(reads)):
                start_read(unit, d)

        def step(h, carry):
            entry = h & (RING - 1)
            pltpu.make_async_copy(in_buf.at[entry], in_buf.at[entry], sems.at[entry]).wait()

            first, end = units_started_before(h), units_started_before(h + 1)

            def start_reads(share):
                for d in range(read_slots * share // B, read_slots * (share + 1) // B):
                    unit = first + d // len(reads)
                    pl.when(unit < end)(functools.partial(
                        start_read, jnp.minimum(unit, n_units - 1), d % len(reads)))

            pending = None
            for b in range(B):
                if b == WRITE_SLOT:
                    for i in range(WRITE_RATE):
                        done = (h - READ_STEPS) * WRITE_RATE + i
                        pl.when(jnp.logical_and(done >= 0, done < h))(
                            functools.partial(start_write, jnp.clip(done, 0, H - 1)))
                if b > 0:
                    start_reads(b - 1)
                    out_buf[b - 1, h] = pending
                qkv = [in_buf[entry, b, pl.ds(row0[t], seq[t])] for t in range(3)]
                pending = _attend(*qkv, scale_log2e).astype(out_buf.dtype)
            start_reads(B - 1)
            out_buf[B - 1, h] = pending
            return carry

        lax.fori_loop(0, H, step, None)

        for done in range(min(H - 1, (H - READ_STEPS) * WRITE_RATE), H):
            start_write(done)
        pltpu.make_async_copy(out_buf, o_hbm, write_sem).wait()

    return pl.pallas_call(
        kernel_function,
        in_specs=[pl.BlockSpec(memory_space=pl.ANY)] * 3,
        out_specs=pl.BlockSpec(memory_space=pl.ANY),
        out_shape=jax.ShapeDtypeStruct(q.shape, q.dtype),
        scratch_shapes=[
            pltpu.VMEM((RING, B, Sq + 2 * Sk, D), q.dtype),
            pltpu.VMEM((B, H, Sq, D), q.dtype),
            pltpu.SemaphoreType.DMA((RING + 1,)),
        ],
        compiler_params=pltpu.CompilerParams(
            vmem_limit_bytes=100 * 1024 * 1024,
            disable_bounds_checks=True,
            disable_semaphore_checks=True,
            flags={"XLA_TPU_MAX_INSTS_TO_PREDICATE": 65536},
        ),
    )(q, k, v)
```
